```python
import jax
import jax.numpy as jnp

def _softmax(x, axis=-1):
    return jax.nn.softmax(x, axis=axis)

def _gelu(x):
    return jax.nn.gelu(x, approximate=True)

def _silu(x):
    return jax.nn.silu(x)

def _sigmoid(x):
    return jax.nn.sigmoid(x)

def _layernorm(x, axis=-1, eps=1e-05):
    m = jnp.mean(x, axis=axis, keepdims=True)
    v = jnp.var(x, axis=axis, keepdims=True)
    return (x - m) / jnp.sqrt(v + eps)

def _scatter_add(tgt, idx, src, axis=0):
    return tgt.at[idx].add(src)

def _segment_sum(src, seg, n):
    return jax.ops.segment_sum(src, seg, n)

class _Rng:

    def __init__(self, key):
        self._k = key

    def _next(self):
        self._k, sub = jax.random.split(self._k)
        return sub

    def normal(self, shape):
        return jax.random.normal(self._next(), shape, dtype=jnp.bfloat16)

    def randint(self, lo, hi, shape):
        return jax.random.randint(self._next(), shape, lo, hi, dtype=jnp.int32)

    def uniform(self, shape, lo=0.0, hi=1.0):
        return jax.random.uniform(self._next(), shape, jnp.bfloat16, lo, hi)

    def permutation(self, n):
        return jax.random.permutation(self._next(), n)
kernel_name = 'adaLN_cond__sliding_block_cached__glu_gated_swiglu__decode'

def setup_inputs():
    _rng = _Rng(jax.random.key(int.from_bytes(__import__("os").urandom(4), "little")))
    _w = lambda a: (lambda t: t.astype(jnp.bfloat16) if jnp.issubdtype(t.dtype, jnp.floating) else t)(jnp.asarray(a))

    def _A_setup():
        B, Sq, D = (2, 1, 512)
        Hq, Hkv, Sk, Dh = (32, 32, 16384, 128)
        assert Hq % Hkv == 0, (Hq, Hkv)
        return {'x': _w((lambda *s: _rng.normal(s) * 0.05)(B, Sq, D)), 'k_cache': _w((lambda *s: _rng.normal(s) * 0.05)(B, Hkv, Sk, Dh)), 'v_cache': _w((lambda *s: _rng.normal(s) * 0.05)(B, Hkv, Sk, Dh)), 'wq': _w((lambda *s: _rng.normal(s) * 0.05)(D, Hq * Dh) * D ** (-0.5)), 'wo': _w((lambda *s: _rng.normal(s) * 0.05)(Hq * Dh, D) * (Hq * Dh) ** (-0.5))}
    _A_in = _A_setup()

    def _B_setup():
        B, S, D, F = (2, 1, 512, 1376)
        return {'x': _w((lambda *s: _rng.normal(s) * 0.05)(B, S, D)), 'w1': _w((lambda *s: _rng.normal(s) * 0.05)(D, F) * (2.0 / D) ** 0.5), 'w3': _w((lambda *s: _rng.normal(s) * 0.05)(D, F) * (2.0 / D) ** 0.5), 'w2': _w((lambda *s: _rng.normal(s) * 0.05)(F, D) * (2.0 / F) ** 0.5)}
    _B_in = _B_setup()
    return {'A_x': _A_in['x'], 'A_k_cache': _A_in['k_cache'], 'A_v_cache': _A_in['v_cache'], 'A_wq': _A_in['wq'], 'A_wo': _A_in['wo'], 'B_x': _B_in['x'], 'B_w1': _B_in['w1'], 'B_w3': _B_in['w3'], 'B_w2': _B_in['w2'], 'c': _w((lambda *s: _rng.normal(s) * 0.05)(2, 512)), 'w_mod': _w((lambda *s: _rng.normal(s) * 0.05)(512, 6 * 512) * 512 ** (-0.5))}

def reference(A_x, A_k_cache, A_v_cache, A_wq, A_wo, B_x, B_w1, B_w3, B_w2, c, w_mod):

    def _A_ref(x, k_cache, v_cache, wq, wo):
        B, Sq, D = x.shape
        Hq, Dh = (32, 128)
        Hkv, Sk = (k_cache.shape[1], k_cache.shape[2])
        W = min(4096, max(256, Sk // 4))
        rep = Hq // Hkv
        q = (lambda x, *d: x.transpose(*d))((x @ wq).reshape(B, Sq, Hq, Dh), 0, 2, 1, 3)
        k = jnp.repeat(k_cache[:, :, Sk - W:, :], rep, axis=1)
        v = jnp.repeat(v_cache[:, :, Sk - W:, :], rep, axis=1)
        scores = jnp.einsum('bhqd,bhkd->bhqk', q, k) * Dh ** (-0.5)
        p = _softmax(scores, axis=-1)
        o = jnp.einsum('bhqk,bhkd->bhqd', p, v)
        return (lambda x, *d: x.transpose(*d))(o, 0, 2, 1, 3).reshape(B, Sq, Hq * Dh) @ wo

    def _B_ref(x, w1, w3, w2):
        gate = jnp.einsum('bsd,df->bsf', x, w1)
        up = jnp.einsum('bsd,df->bsf', x, w3)
        h = _silu(gate) * up
        out = jnp.einsum('bsf,fd->bsd', h, w2)
        return out
    x = A_x
    mod = (_silu(c) @ w_mod).reshape(c.shape[0], 6, 1, -1)
    sa, ca, ga, sb, cb, gb = (mod[:, 0].copy(), mod[:, 1].copy(), mod[:, 2].copy(), mod[:, 3].copy(), mod[:, 4].copy(), mod[:, 5].copy())
    h = _layernorm(x, axis=-1) * (1 + ca) + sa
    x = x + ga * _A_ref(h, A_k_cache, A_v_cache, A_wq, A_wo)
    h = _layernorm(x, axis=-1) * (1 + cb) + sb
    x = x + gb * _B_ref(h, B_w1, B_w3, B_w2)
    return x
```

```python
import functools
import jax, jax.numpy as jnp
from jax import lax
from jax.experimental import pallas as pl
from jax.experimental.pallas import tpu as pltpu

B, D, HQ, DH, SK, F = 2, 512, 32, 128, 16384, 1376
W = min(4096, max(256, SK // 4))
G = 4
NG = HQ // G
BF, F32 = jnp.bfloat16, jnp.float32
NT = (((1,), (1,)), ((), ()))

def make(R=128, DEPTH=8, hstride=8, skew=0, name="k1", nobc=True, compute=True):
    CPH = W // R
    NSTEP = NG * CPH

    def head_of(g, hh):
        if hstride == 1:
            return g * G + hh
        return (g // hstride) * (hstride * G) + (g % hstride) + hh * hstride

    def kernel(x_hbm, c_hbm, k_hbm, v_hbm, wq_hbm, wo_hbm, w1_hbm, w3_hbm, w2_hbm, wm_hbm, o_hbm,
               x_v, c_v, o_v, buf, wq_v, wo_v, w1_v, w3_v, w2_v, wm_v, q_s, o_s, sems, wsem):
        def start(t, slot):
            g = t // CPH
            c = t % CPH
            for hh in range(G):
                h = head_of(g, hh)
                cc = (c + skew * hh) % CPH if skew else c
                off = pl.multiple_of(SK - W + cc * R, R)
                for kv, src in enumerate((k_hbm, v_hbm)):
                    for b in range(B):
                        pltpu.make_async_copy(src.at[b, h, pl.ds(off, R), :], buf.at[slot, b, 2 * hh + kv],
                                              sems.at[slot, b]).start(priority=b)
        def wait(slot):
            for b in range(B):
                pltpu.make_async_copy(buf.at[slot, b], buf.at[slot, b], sems.at[slot, b]).wait()

        names = [(c_hbm, c_v), (x_hbm, x_v), (wm_hbm, wm_v), (wq_hbm, wq_v), (wo_hbm, wo_v), (w1_hbm, w1_v), (w3_hbm, w3_v), (w2_hbm, w2_v)]
        cp = [pltpu.make_async_copy(a, b_, wsem.at[j]) for j, (a, b_) in enumerate(names)]
        cp[0].start(); cp[1].start(priority=1); cp[2].start(); cp[3].start(priority=1)
        for s in range(DEPTH):
            start(s, s)

        row = lax.broadcasted_iota(jnp.int32, (8, 128), 0)
        roww = lax.broadcasted_iota(jnp.int32, (8, D), 0)
        def rep8(ref):
            v = ref[...].astype(F32)
            return jnp.where(roww % 2 == 0, v[0:1], v[1:2])
        def ln(v):
            m = jnp.mean(v, axis=-1, keepdims=True)
            d = v - m
            var = jnp.mean(d * d, axis=-1, keepdims=True)
            return d * lax.rsqrt(var + 1e-5)

        cp[0].wait(); cp[2].wait()
        c8 = rep8(c_v)
        sc = (c8 * jax.nn.sigmoid(c8)).astype(BF)
        mod = jnp.dot(sc, wm_v[...], preferred_element_type=F32)
        sa, ca, ga, sb, cb, gb = [mod[:, i * D:(i + 1) * D] for i in range(6)]
        cp[1].wait()
        x8 = rep8(x_v)
        h = (ln(x8) * (1 + ca) + sa).astype(BF)
        cp[3].wait()
        q = jnp.dot(h, wq_v[...], preferred_element_type=F32)
        for hd in range(HQ):
            q_s[hd] = q[:, hd * DH:(hd + 1) * DH]
        scale = DH ** -0.5

        def group(g, _):
            qs = [q_s[head_of(g, hh)].astype(BF) for hh in range(G)]
            def step(c, carry):
                m, l, acc = carry
                t = g * CPH + c
                slot = t % DEPTH
                wait(slot)
                if compute:
                    s = None
                    for hh in range(G):
                        for b in range(B):
                            r = lax.dot_general(qs[hh], buf[slot, b, 2 * hh], NT, preferred_element_type=F32)
                            rr = lax.broadcasted_iota(jnp.int32, r.shape, 0)
                            s = r if s is None else jnp.where(rr == 2 * hh + b, r, s)
                    s = s * scale
                    m_new = jnp.maximum(m, jnp.max(s, axis=-1, keepdims=True))
                    alpha = jnp.exp(m - m_new)
                    p = jnp.exp(s - m_new)
                    l = alpha * l + jnp.sum(p, axis=-1, keepdims=True)
                    pb = p.astype(BF)
                    o = None
                    for hh in range(G):
                        for b in range(B):
                            r = jnp.dot(pb, buf[slot, b, 2 * hh + 1], preferred_element_type=F32)
                            o = r if o is None else jnp.where(row == 2 * hh + b, r, o)
                    acc = alpha * acc + o
                    m = m_new
                @pl.when(t + DEPTH < NSTEP)
                def _():
                    start(t + DEPTH, slot)
                @pl.when(t + DEPTH == NSTEP)
                def _():
                    cp[4].start(); cp[5].start(priority=1); cp[6].start(priority=1); cp[7].start()
                return m, l, acc
            m0 = jnp.full((8, 1), -jnp.inf, F32)
            m, l, acc = lax.fori_loop(0, CPH, step, (m0, jnp.zeros((8, 1), F32), jnp.zeros((8, DH), F32)))
            o = acc / l
            for hh in range(G):
                o_s[head_of(g, hh)] = jnp.where(row // 2 == hh, o, 0.0)
            return 0
        lax.fori_loop(0, NG, group, 0)

        cp[4].wait()
        ocat = jnp.concatenate([o_s[hd] for hd in range(HQ)], axis=-1).astype(BF)
        a = jnp.dot(ocat, wo_v[...], preferred_element_type=F32)
        a = a + pltpu.roll(a, 4, 0)
        a = a + pltpu.roll(a, 2, 0)
        x1 = x8 + ga * a
        h2 = (ln(x1) * (1 + cb) + sb).astype(BF)
        cp[5].wait(); cp[6].wait()
        gate = lax.dot_general(h2, w1_v[...], NT, preferred_element_type=F32)
        up = lax.dot_general(h2, w3_v[...], NT, preferred_element_type=F32)
        act = (gate * jax.nn.sigmoid(gate) * up).astype(BF)
        cp[7].wait()
        y = jnp.dot(act, w2_v[...], preferred_element_type=F32)
        out = x1 + gb * y
        o_v[...] = out[0:2].astype(BF)
        oc = pltpu.make_async_copy(o_v, o_hbm, wsem.at[0]); oc.start(); oc.wait()

    def fn(A_x, A_k_cache, A_v_cache, A_wq, A_wo, B_x, B_w1, B_w3, B_w2, c, w_mod):
        hbm = pl.BlockSpec(memory_space=pltpu.HBM)
        out = pl.pallas_call(
            kernel, out_shape=jax.ShapeDtypeStruct((B, D), BF),
            in_specs=[hbm] * 10, out_specs=hbm,
            scratch_shapes=[
                pltpu.VMEM((B, D), BF), pltpu.VMEM((B, D), BF), pltpu.VMEM((B, D), BF),
                pltpu.VMEM((DEPTH, B, 2 * G, R, DH), BF),
                pltpu.VMEM((D, HQ * DH), BF), pltpu.VMEM((HQ * DH, D), BF),
                pltpu.VMEM((F, D), BF), pltpu.VMEM((F, D), BF), pltpu.VMEM((F, D), BF),
                pltpu.VMEM((D, 6 * D), BF),
                pltpu.VMEM((HQ, 8, DH), F32), pltpu.VMEM((HQ, 8, DH), F32),
                pltpu.SemaphoreType.DMA((DEPTH, 2)), pltpu.SemaphoreType.DMA((8,))],
            compiler_params=pltpu.CompilerParams(vmem_limit_bytes=100 * 1024 * 1024, disable_bounds_checks=nobc),
            name=name,
        )(A_x.reshape(B, D), c, A_k_cache, A_v_cache, A_wq, A_wo, B_w1.T, B_w3.T, B_w2, w_mod)
        return out.reshape(B, 1, D)
    return fn


_impl = make(R=128, DEPTH=8, hstride=8, name="adaln_swa_swiglu_decode")


@jax.jit
def pallas_adaLN_cond__sliding_block_cached__glu_gated_swiglu__decode_kernel(
    A_x: jax.Array,
    A_k_cache: jax.Array,
    A_v_cache: jax.Array,
    A_wq: jax.Array,
    A_wo: jax.Array,
    B_x: jax.Array,
    B_w1: jax.Array,
    B_w3: jax.Array,
    B_w2: jax.Array,
    c: jax.Array,
    w_mod: jax.Array,
):
    return _impl(A_x, A_k_cache, A_v_cache, A_wq, A_wo, B_x, B_w1, B_w3, B_w2, c, w_mod)
```

```python
import itertools
import jax, jax.numpy as jnp
from jax import lax
from jax.experimental import pallas as pl
from jax.experimental.pallas import tpu as pltpu

B, D, HQ, DH, SK, F = 2, 512, 32, 128, 16384, 1376
W = min(4096, max(256, SK // 4))
G = 4
NG = HQ // G
R = 128
HR = R // 2
CPH = W // R
NSTEP = NG * CPH
BF, F32 = jnp.bfloat16, jnp.float32
NT = (((1,), (1,)), ((), ()))


def make(NS=8, hstride=4, ko=0, vo=1, FC=(384, 384, 384, 224), name="k4", nobc=True,
         wmP=(8, 1536, 4), wqP=(8, 2048, 4), woP=(32, 0, 4), fP=(32, 0, 0, 0)):
    shift = (ko, vo)
    lag = 1 if (ko or vo) else 0
    DEPTH = NS - lag
    assert sum(FC) == F
    FO = [sum(FC[:i]) for i in range(len(FC))]

    def head_of(g, hh):
        return (g // hstride) * (hstride * G) + (g % hstride) + hh * hstride

    def kernel(x_hbm, c_hbm, k_hbm, v_hbm, wq_hbm, wo_hbm, w1_hbm, w3_hbm, w2_hbm, wm_hbm, o_hbm,
               x_v, c_v, o_v, buf, wq_v, wo_v, w1_v, w3_v, w2_v, wm_v, q_s, sems, wsem, fsem):
        kv_hbm = (k_hbm, v_hbm)

        def dma(kv, b, head, r0, n, slot, hh, d0):
            pltpu.make_async_copy(kv_hbm[kv].at[b, head, pl.ds(r0, n), :], buf.at[slot, b, kv, hh, pl.ds(d0, n), :],
                                  sems.at[slot, b, kv]).start(priority=b)

        def start(t, slot):
            static = isinstance(t, int)
            g = t // CPH
            c = t % CPH
            off = SK - W + c * R
            if not static:
                off = pl.multiple_of(off, R)
            def regular():
                for hh in range(G):
                    for kv in range(2):
                        for b in range(B):
                            dma(kv, b, head_of(g, hh), off + HR * shift[kv], R, slot, hh, 0)
            def last(nxt):
                for hh in range(G):
                    for kv in range(2):
                        for b in range(B):
                            if shift[kv]:
                                dma(kv, b, head_of(g, hh), SK - HR, HR, slot, hh, 0)
                                if nxt:
                                    dma(kv, b, head_of(g + 1, hh), SK - W, HR, slot, hh, HR)
                            else:
                                dma(kv, b, head_of(g, hh), SK - R, R, slot, hh, 0)
            if not lag:
                regular()
            elif static:
                assert c < CPH - 1
                regular()
            else:
                pl.when(c < CPH - 1)(regular)
                @pl.when(c == CPH - 1)
                def _():
                    pl.when(g < NG - 1)(lambda: last(True))
                    pl.when(g == NG - 1)(lambda: last(False))

        def wait(t, slot):
            for b in range(B):
                for kv in range(2):
                    full = buf.at[slot, b, kv]
                    if shift[kv]:
                        half = buf.at[slot, b, kv, :, pl.ds(0, HR), :]
                        pl.when(t < NSTEP - 1)(lambda: pltpu.make_async_copy(full, full, sems.at[slot, b, kv]).wait())
                        pl.when(t == NSTEP - 1)(lambda: pltpu.make_async_copy(half, half, sems.at[slot, b, kv]).wait())
                    else:
                        pltpu.make_async_copy(full, full, sems.at[slot, b, kv]).wait()

        def tile(slot, prev, hh, kv, b):
            if shift[kv]:
                return jnp.concatenate([buf[prev, b, kv, hh, pl.ds(HR, HR), :], buf[slot, b, kv, hh, pl.ds(0, HR), :]], axis=0)
            return buf[slot, b, kv, hh]

        qcount = [0]
        def interleave(lists):
            return [p for tup in itertools.zip_longest(*lists) for p in tup if p is not None]
        def streams(ps, s):
            n = -(-len(ps) // s)
            return interleave([ps[i * n:(i + 1) * n] for i in range(s)])
        def rowpieces(a, b_, sem, r0, nr, cr, first=0):
            cuts = [r0] + [r for r in range(first if first else cr, a.shape[0], cr) if r0 < r < r0 + nr] + [r0 + nr]
            return [(a.at[pl.ds(lo, hi - lo)], b_.at[pl.ds(lo, hi - lo)], sem) for lo, hi in zip(cuts[:-1], cuts[1:])]
        def tilepieces(a, b_, sem, cr, cc):
            return [(a.at[pl.ds(r, cr), pl.ds(c_, cc)], b_.at[pl.ds(r, cr), pl.ds(c_, cc)], sem)
                    for r in range(0, a.shape[0], cr) for c_ in range(0, a.shape[1], cc)]
        def pstart(ps):
            for p in ps:
                pltpu.make_async_copy(*p).start(priority=qcount[0] % 2)
                qcount[0] += 1
        def wwait(v, sem):
            pltpu.make_async_copy(v, v, sem).wait()

        cc = pltpu.make_async_copy(c_hbm, c_v, wsem.at[0])
        xc = pltpu.make_async_copy(x_hbm, x_v, wsem.at[1])
        pstart(streams(tilepieces(wm_hbm, wm_v, wsem.at[2], wmP[0], wmP[1]), wmP[2]))
        cc.start(); xc.start(priority=1)
        pstart(streams(tilepieces(wq_hbm, wq_v, wsem.at[3], wqP[0], wqP[1]), wqP[2]))
        fps = []
        for j, (f0, fc) in enumerate(zip(FO, FC)):
            fps += interleave([rowpieces(w1_hbm, w1_v, fsem.at[0, j], f0, fc, fP[0], fP[1]),
                               rowpieces(w3_hbm, w3_v, fsem.at[1, j], f0, fc, fP[0], fP[2])])
        for j, (f0, fc) in enumerate(zip(FO, FC)):
            fps += rowpieces(w2_hbm, w2_v, fsem.at[2, j], f0, fc, fP[0], fP[3])
        nb = -(-len(fps) // DEPTH)
        fbatches = [fps[i * nb:(i + 1) * nb] for i in range(DEPTH)]

        row = lax.broadcasted_iota(jnp.int32, (8, 128), 0)
        roww = lax.broadcasted_iota(jnp.int32, (8, D), 0)
        def rep8(ref):
            v = ref[...].astype(F32)
            return jnp.where(roww % 2 == 0, v[0:1], v[1:2])
        def ln(v):
            m = jnp.mean(v, axis=-1, keepdims=True)
            d = v - m
            var = jnp.mean(d * d, axis=-1, keepdims=True)
            return d * lax.rsqrt(var + 1e-5)

        cc.wait()
        c8 = rep8(c_v)
        sc = (c8 * jax.nn.sigmoid(c8)).astype(BF)
        xc.wait()
        x8 = rep8(x_v)
        wwait(wm_v, wsem.at[2])
        mod = jnp.dot(sc, wm_v[...], preferred_element_type=F32)
        sa, ca, ga, sb, cb, gb = [mod[:, i * D:(i + 1) * D] for i in range(6)]
        h = (ln(x8) * (1 + ca) + sa).astype(BF)
        for kv in range(2):
            if shift[kv]:
                for hh in range(G):
                    for b in range(B):
                        dma(kv, b, head_of(0, hh), SK - W, HR, NS - 1, hh, HR)
        for s in range(DEPTH):
            start(s, s)
        wwait(wq_v, wsem.at[3])
        q = jnp.dot(h, wq_v[...], preferred_element_type=F32)
        for hd in range(HQ):
            q_s[hd] = q[:, hd * DH:(hd + 1) * DH]
        pstart(streams(rowpieces(wo_hbm, wo_v, wsem.at[4], 0, HQ * DH, woP[0], woP[1]), woP[2]))
        for kv in range(2):
            if shift[kv]:
                for b in range(B):
                    wwait(buf.at[NS - 1, b, kv, :, pl.ds(HR, HR), :], sems.at[NS - 1, b, kv])
        scale = DH ** -0.5

        def group(g, attn):
            qs = [q_s[head_of(g, hh)].astype(BF) for hh in range(G)]
            def step(c, carry):
                m, l, acc = carry
                t = g * CPH + c
                slot = t % NS
                prev = (t + NS - 1) % NS
                wait(t, slot)
                s = None
                for hh in range(G):
                    for b in range(B):
                        r = lax.dot_general(qs[hh], tile(slot, prev, hh, 0, b), NT, preferred_element_type=F32)
                        s = r if s is None else jnp.where(row == 2 * hh + b, r, s)
                s = s * scale
                m_new = jnp.maximum(m, jnp.max(s, axis=-1, keepdims=True))
                alpha = jnp.exp(m - m_new)
                p = jnp.exp(s - m_new)
                l = alpha * l + jnp.sum(p, axis=-1, keepdims=True)
                pb = p.astype(BF)
                o = None
                for hh in range(G):
                    for b in range(B):
                        r = jnp.dot(pb, tile(slot, prev, hh, 1, b), preferred_element_type=F32)
                        o = r if o is None else jnp.where(row == 2 * hh + b, r, o)
                acc = alpha * acc + o
                @pl.when(t + DEPTH < NSTEP)
                def _():
                    start(t + DEPTH, prev if lag else slot)
                @pl.when(t + DEPTH >= NSTEP)
                def _():
                    for j in range(DEPTH):
                        @pl.when(t + DEPTH == NSTEP + j)
                        def _():
                            pstart(fbatches[j])
                return m_new, l, acc
            m0 = jnp.full((8, 1), -jnp.inf, F32)
            m, l, acc = lax.fori_loop(0, CPH, step, (m0, jnp.zeros((8, 1), F32), jnp.zeros((8, DH), F32)))
            o = acc / l
            @pl.when(g == 0)
            def _():
                wwait(wo_v, wsem.at[4])
            for hh in range(G):
                lhs = jnp.where(row // 2 == hh, o, 0.0).astype(BF)
                r0 = pl.multiple_of(head_of(g, hh) * DH, DH)
                attn = attn + jnp.dot(lhs, wo_v[pl.ds(r0, DH), :], preferred_element_type=F32)
            return attn
        a = lax.fori_loop(0, NG, group, jnp.zeros((8, D), F32))

        a = a + pltpu.roll(a, 4, 0)
        a = a + pltpu.roll(a, 2, 0)
        x1 = x8 + ga * a
        h2 = (ln(x1) * (1 + cb) + sb).astype(BF)
        acts = []
        for j, (f0, fc) in enumerate(zip(FO, FC)):
            wwait(w1_v.at[pl.ds(f0, fc)], fsem.at[0, j])
            wwait(w3_v.at[pl.ds(f0, fc)], fsem.at[1, j])
            gate = lax.dot_general(h2, w1_v[pl.ds(f0, fc), :], NT, preferred_element_type=F32)
            up = lax.dot_general(h2, w3_v[pl.ds(f0, fc), :], NT, preferred_element_type=F32)
            acts.append((gate * jax.nn.sigmoid(gate) * up).astype(BF))
        y = None
        for j, (f0, fc) in enumerate(zip(FO, FC)):
            wwait(w2_v.at[pl.ds(f0, fc)], fsem.at[2, j])
            r = jnp.dot(acts[j], w2_v[pl.ds(f0, fc), :], preferred_element_type=F32)
            y = r if y is None else y + r
        out = x1 + gb * y
        o_v[...] = out[0:2].astype(BF)
        oc = pltpu.make_async_copy(o_v, o_hbm, wsem.at[5]); oc.start(); oc.wait()

    def fn(A_x, A_k_cache, A_v_cache, A_wq, A_wo, B_x, B_w1, B_w3, B_w2, c, w_mod):
        hbm = pl.BlockSpec(memory_space=pltpu.HBM)
        out = pl.pallas_call(
            kernel, out_shape=jax.ShapeDtypeStruct((B, D), BF),
            in_specs=[hbm] * 10, out_specs=hbm,
            scratch_shapes=[
                pltpu.VMEM((B, D), BF), pltpu.VMEM((B, D), BF), pltpu.VMEM((B, D), BF),
                pltpu.VMEM((NS, B, 2, G, R, DH), BF),
                pltpu.VMEM((D, HQ * DH), BF), pltpu.VMEM((HQ * DH, D), BF),
                pltpu.VMEM((F, D), BF), pltpu.VMEM((F, D), BF), pltpu.VMEM((F, D), BF),
                pltpu.VMEM((D, 6 * D), BF),
                pltpu.VMEM((HQ, 8, DH), F32),
                pltpu.SemaphoreType.DMA((NS, B, 2)), pltpu.SemaphoreType.DMA((6,)), pltpu.SemaphoreType.DMA((3, len(FC)))],
            compiler_params=pltpu.CompilerParams(vmem_limit_bytes=100 * 1024 * 1024, disable_bounds_checks=nobc),
            name=name,
        )(A_x.reshape(B, D), c, A_k_cache, A_v_cache, A_wq, A_wo, B_w1.T, B_w3.T, B_w2, w_mod)
        return out.reshape(B, 1, D)
    return fn


_impl = make(NS=7, name="adaln_swa_swiglu_decode")


@jax.jit
def pallas_adaLN_cond__sliding_block_cached__glu_gated_swiglu__decode_kernel(
    A_x: jax.Array,
    A_k_cache: jax.Array,
    A_v_cache: jax.Array,
    A_wq: jax.Array,
    A_wo: jax.Array,
    B_x: jax.Array,
    B_w1: jax.Array,
    B_w3: jax.Array,
    B_w2: jax.Array,
    c: jax.Array,
    w_mod: jax.Array,
):
    return _impl(A_x, A_k_cache, A_v_cache, A_wq, A_wo, B_x, B_w1, B_w3, B_w2, c, w_mod)
```

```python
import itertools

import jax
import jax.numpy as jnp
from jax import lax
import jax.experimental.pallas as pl
import jax.experimental.pallas.tpu as pltpu

B, D, HQ, DH, SK, F = 2, 512, 32, 128, 16384, 1376
W = min(4096, max(256, SK // 4))
BF, F32 = jnp.bfloat16, jnp.float32
NT = (((1,), (1,)), ((), ()))

G = 4
NG = HQ // G
HSTRIDE = 4
R = 128
HR = R // 2
CPH = W // R
NSTEP = NG * CPH
NS = 7
DEPTH = NS - 1
W2_CHUNKS = (1024, 256, 96)
assert sum(W2_CHUNKS) == F and W % R == 0


def _head_of(g, hh):
    return (g // HSTRIDE) * (HSTRIDE * G) + (g % HSTRIDE) + hh * HSTRIDE


def _interleave(lists):
    return [p for tup in itertools.zip_longest(*lists) for p in tup if p is not None]


def _streams(pieces, n):
    k = -(-len(pieces) // n)
    return _interleave([pieces[i * k:(i + 1) * k] for i in range(n)])


def _pieces(src, dst, sem, rows, cols, r0=0, nrows=None):
    r1 = src.shape[0] if nrows is None else r0 + nrows
    out = []
    for r in range(r0, r1, rows):
        n = min(rows, r1 - r)
        for c in range(0, src.shape[1], cols):
            out.append(pltpu.make_async_copy(src.at[pl.ds(r, n), pl.ds(c, cols)],
                                             dst.at[pl.ds(r, n), pl.ds(c, cols)], sem))
    return out


def _with_queues(pieces, num, den):
    return [(p, 0 if (i * num) % den < num else 1) for i, p in enumerate(pieces)]


def _start_all(pieces_with_queues):
    for p, q in pieces_with_queues:
        p.start(priority=q)


def _wait_filled(dst, sem):
    pltpu.make_async_copy(dst, dst, sem).wait()


def _layernorm(v):
    d = v - jnp.mean(v, axis=-1, keepdims=True)
    var = jnp.mean(d * d, axis=-1, keepdims=True)
    return d * lax.rsqrt(var + 1e-5)


def _kernel(x_hbm, c_hbm, k_hbm, v_hbm, wq_hbm, wo_hbm, w1t_hbm, w3t_hbm, w2_hbm, wm_hbm, o_hbm,
            x_v, c_v, o_v, ring, wq_v, wo_v, w1_v, w3_v, w2_v, wm_v, q_s, rsem, wsem):
    def kv_start(kv, b, head, r0, n, slot, hh, d0):
        src = (k_hbm, v_hbm)[kv].at[b, head, pl.ds(r0, n), :]
        dst = ring.at[slot, kv, b, hh, pl.ds(d0, n), :]
        pltpu.make_async_copy(src, dst, rsem.at[slot, kv]).start(priority=b)

    def ring_start(t, slot):
        g, c = t // CPH, t % CPH
        off = SK - W + c * R

        def inner_chunk():
            for hh in range(G):
                for kv in range(2):
                    for b in range(B):
                        kv_start(kv, b, _head_of(g, hh), off + HR * kv, R, slot, hh, 0)

        def last_chunk(has_next_group):
            for hh in range(G):
                for b in range(B):
                    kv_start(0, b, _head_of(g, hh), SK - R, R, slot, hh, 0)
                for b in range(B):
                    kv_start(1, b, _head_of(g, hh), SK - HR, HR, slot, hh, 0)
                    if has_next_group:
                        kv_start(1, b, _head_of(g + 1, hh), SK - W, HR, slot, hh, HR)

        if isinstance(t, int):
            assert c < CPH - 1
            inner_chunk()
        else:
            off = pl.multiple_of(off, R)
            pl.when(c < CPH - 1)(inner_chunk)

            @pl.when(c == CPH - 1)
            def _():
                pl.when(g < NG - 1)(lambda: last_chunk(True))
                pl.when(g == NG - 1)(lambda: last_chunk(False))

    def ring_wait(t, slot):
        _wait_filled(ring.at[slot, 0], rsem.at[slot, 0])
        pl.when(t < NSTEP - 1)(lambda: _wait_filled(ring.at[slot, 1], rsem.at[slot, 1]))
        pl.when(t == NSTEP - 1)(
            lambda: _wait_filled(ring.at[slot, 1, :, :, pl.ds(0, HR), :], rsem.at[slot, 1]))

    c_copy = pltpu.make_async_copy(c_hbm, c_v, wsem.at[0])
    x_copy = pltpu.make_async_copy(x_hbm, x_v, wsem.at[1])
    _start_all(_with_queues(_streams(_pieces(wm_hbm, wm_v, wsem.at[2], 8, 1536), 4), 1, 2))
    c_copy.start()
    x_copy.start(priority=1)
    _start_all(_with_queues(_streams(_pieces(wq_hbm, wq_v, wsem.at[3], 8, 2048), 4), 1, 2))

    w2_offsets = [sum(W2_CHUNKS[:j]) for j in range(len(W2_CHUNKS))]
    ffn = _with_queues(_interleave([_streams(_pieces(w1t_hbm, w1_v, wsem.at[0], 32, D), 2),
                                    _streams(_pieces(w3t_hbm, w3_v, wsem.at[1], 32, D), 2)]), 5, 8)
    for j, (f0, fc) in enumerate(zip(w2_offsets, W2_CHUNKS)):
        ffn += _with_queues(_pieces(w2_hbm, w2_v, wsem.at[2 + j], 32, D, f0, fc), 0, 1)
    per_step = -(-len(ffn) // DEPTH)
    ffn_batches = [ffn[j * per_step:(j + 1) * per_step] for j in range(DEPTH)]

    row = lax.broadcasted_iota(jnp.int32, (8, DH), 0)
    row_d = lax.broadcasted_iota(jnp.int32, (8, D), 0)

    def rows8(ref):
        v = ref[...].astype(F32)
        return jnp.where(row_d % 2 == 0, v[0:1], v[1:2])

    c_copy.wait()
    c8 = rows8(c_v)
    silu_c = (c8 * jax.nn.sigmoid(c8)).astype(BF)
    x_copy.wait()
    x8 = rows8(x_v)
    _wait_filled(wm_v, wsem.at[2])
    mod = jnp.dot(silu_c, wm_v[...], preferred_element_type=F32)
    sa, ca, ga, sb, cb, gb = [mod[:, i * D:(i + 1) * D] for i in range(6)]
    h = (_layernorm(x8) * (1 + ca) + sa).astype(BF)

    for hh in range(G):
        for b in range(B):
            kv_start(1, b, _head_of(0, hh), SK - W, HR, NS - 1, hh, HR)
    for t in range(DEPTH):
        ring_start(t, t)
    _wait_filled(wq_v, wsem.at[3])
    q = jnp.dot(h, wq_v[...], preferred_element_type=F32)
    for head in range(HQ):
        q_s[head] = q[:, head * DH:(head + 1) * DH]
    _start_all(_with_queues(_streams(_pieces(wo_hbm, wo_v, wsem.at[4], 32, D), 4), 1, 2))
    _wait_filled(ring.at[NS - 1, 1, :, :, pl.ds(HR, HR), :], rsem.at[NS - 1, 1])

    scale = DH ** -0.5

    def group(g, attn):
        qs = [q_s[_head_of(g, hh)].astype(BF) for hh in range(G)]

        def step(c, carry):
            m, l, acc = carry
            t = g * CPH + c
            slot, prev = t % NS, (t + NS - 1) % NS
            ring_wait(t, slot)
            s = None
            for hh in range(G):
                for b in range(B):
                    r = lax.dot_general(qs[hh], ring[slot, 0, b, hh], NT, preferred_element_type=F32)
                    s = r if s is None else jnp.where(row == 2 * hh + b, r, s)
            s = s * scale
            m_new = jnp.maximum(m, jnp.max(s, axis=-1, keepdims=True))
            alpha = jnp.exp(m - m_new)
            p = jnp.exp(s - m_new)
            l = alpha * l + jnp.sum(p, axis=-1, keepdims=True)
            p = p.astype(BF)
            o = None
            for hh in range(G):
                for b in range(B):
                    v = jnp.concatenate([ring[prev, 1, b, hh, pl.ds(HR, HR), :],
                                         ring[slot, 1, b, hh, pl.ds(0, HR), :]], axis=0)
                    r = jnp.dot(p, v, preferred_element_type=F32)
                    o = r if o is None else jnp.where(row == 2 * hh + b, r, o)
            acc = alpha * acc + o

            pl.when(t + DEPTH < NSTEP)(lambda: ring_start(t + DEPTH, prev))

            @pl.when(t + DEPTH >= NSTEP)
            def _():
                for j in range(DEPTH):
                    pl.when(t + DEPTH == NSTEP + j)(lambda j=j: _start_all(ffn_batches[j]))

            return m_new, l, acc

        init = (jnp.full((8, 1), -jnp.inf, F32), jnp.zeros((8, 1), F32), jnp.zeros((8, DH), F32))
        _, l, acc = lax.fori_loop(0, CPH, step, init)
        o = acc / l
        pl.when(g == 0)(lambda: _wait_filled(wo_v, wsem.at[4]))
        for hh in range(G):
            lhs = jnp.where(row // 2 == hh, o, 0.0).astype(BF)
            r0 = pl.multiple_of(_head_of(g, hh) * DH, DH)
            attn = attn + jnp.dot(lhs, wo_v[pl.ds(r0, DH), :], preferred_element_type=F32)
        return attn

    a = lax.fori_loop(0, NG, group, jnp.zeros((8, D), F32))
    a = a + pltpu.roll(a, 4, 0)
    a = a + pltpu.roll(a, 2, 0)

    x1 = x8 + ga * a
    h2 = (_layernorm(x1) * (1 + cb) + sb).astype(BF)
    _wait_filled(w1_v, wsem.at[0])
    _wait_filled(w3_v, wsem.at[1])
    gate = lax.dot_general(h2, w1_v[...], NT, preferred_element_type=F32)
    up = lax.dot_general(h2, w3_v[...], NT, preferred_element_type=F32)
    act = (gate * jax.nn.sigmoid(gate) * up).astype(BF)
    y = None
    for j, (f0, fc) in enumerate(zip(w2_offsets, W2_CHUNKS)):
        _wait_filled(w2_v.at[pl.ds(f0, fc), :], wsem.at[2 + j])
        r = jnp.dot(act[:, f0:f0 + fc], w2_v[pl.ds(f0, fc), :], preferred_element_type=F32)
        y = r if y is None else y + r
    out = x1 + gb * y
    o_v[...] = out[0:B].astype(BF)
    o_copy = pltpu.make_async_copy(o_v, o_hbm, wsem.at[0])
    o_copy.start()
    o_copy.wait()


@jax.jit
def pallas_adaLN_cond__sliding_block_cached__glu_gated_swiglu__decode_kernel(
    A_x: jax.Array,
    A_k_cache: jax.Array,
    A_v_cache: jax.Array,
    A_wq: jax.Array,
    A_wo: jax.Array,
    B_x: jax.Array,
    B_w1: jax.Array,
    B_w3: jax.Array,
    B_w2: jax.Array,
    c: jax.Array,
    w_mod: jax.Array,
):
    del B_x
    assert A_x.shape == (B, 1, D) and A_k_cache.shape == A_v_cache.shape == (B, HQ, SK, DH)
    hbm = pl.BlockSpec(memory_space=pltpu.HBM)
    out = pl.pallas_call(
        _kernel,
        out_shape=jax.ShapeDtypeStruct((B, D), BF),
        in_specs=[hbm] * 10,
        out_specs=hbm,
        scratch_shapes=[
            pltpu.VMEM((B, D), BF),
            pltpu.VMEM((B, D), BF),
            pltpu.VMEM((B, D), BF),
            pltpu.VMEM((NS, 2, B, G, R, DH), BF),
            pltpu.VMEM((D, HQ * DH), BF),
            pltpu.VMEM((HQ * DH, D), BF),
            pltpu.VMEM((F, D), BF),
            pltpu.VMEM((F, D), BF),
            pltpu.VMEM((F, D), BF),
            pltpu.VMEM((D, 6 * D), BF),
            pltpu.VMEM((HQ, 8, DH), F32),
            pltpu.SemaphoreType.DMA((NS, 2)),
            pltpu.SemaphoreType.DMA((max(5, 2 + len(W2_CHUNKS)),)),
        ],
        compiler_params=pltpu.CompilerParams(
            vmem_limit_bytes=64 * 1024 * 1024,
            disable_bounds_checks=True,
            disable_semaphore_checks=True,
        ),
        name="adaln_swa_swiglu_decode",
    )(A_x.reshape(B, D), c, A_k_cache, A_v_cache, A_wq, A_wo, B_w1.T, B_w3.T, B_w2, w_mod)
    return out.reshape(B, 1, D)
```

```python
import itertools

import jax
import jax.numpy as jnp
from jax import lax
import jax.experimental.pallas as pl
import jax.experimental.pallas.tpu as pltpu

B, D, HQ, DH, SK, F = 2, 512, 32, 128, 16384, 1376
W = min(4096, max(256, SK // 4))
BF, F32 = jnp.bfloat16, jnp.float32
NT = (((1,), (1,)), ((), ()))

G = 4
NG = HQ // G
HSTRIDE = 4
P = 128
R = 256
SHIFT = (128, 64)
CPH = W // R
NSTEP = NG * CPH
NS = 5
DEPTH = NS - 1
W2_CHUNKS = (1024, 256, 96)
assert sum(W2_CHUNKS) == F and W % R == 0 and R % P == 0

def _head_of(g, hh):
    return (g // HSTRIDE) * (HSTRIDE * G) + (g % HSTRIDE) + hh * HSTRIDE


def _interleave(lists):
    return [p for tup in itertools.zip_longest(*lists) for p in tup if p is not None]


def _streams(pieces, n):
    k = -(-len(pieces) // n)
    return _interleave([pieces[i * k:(i + 1) * k] for i in range(n)])


def _pieces(src, dst, sem, rows, cols, r0=0, nrows=None):
    r1 = src.shape[0] if nrows is None else r0 + nrows
    out = []
    for r in range(r0, r1, rows):
        n = min(rows, r1 - r)
        for c in range(0, src.shape[1], cols):
            out.append(pltpu.make_async_copy(src.at[pl.ds(r, n), pl.ds(c, cols)],
                                             dst.at[pl.ds(r, n), pl.ds(c, cols)], sem))
    return out


def _with_queues(pieces, num, den):
    return [(p, 0 if (i * num) % den < num else 1) for i, p in enumerate(pieces)]


def _start_all(pieces_with_queues):
    for p, q in pieces_with_queues:
        p.start(priority=q)


def _wait_filled(dst, sem):
    pltpu.make_async_copy(dst, dst, sem).wait()


def _layernorm(v):
    d = v - jnp.mean(v, axis=-1, keepdims=True)
    var = jnp.mean(d * d, axis=-1, keepdims=True)
    return d * lax.rsqrt(var + 1e-5)


def _kernel(x_hbm, c_hbm, k_hbm, v_hbm, wq_hbm, wo_hbm, w1t_hbm, w3t_hbm, w2_hbm, wm_hbm, o_hbm,
            x_v, c_v, o_v, ring, wq_v, wo_v, w1_v, w3_v, w2_v, wm_v, q_s, rsem, wsem):
    def kv_start(kv, b, head, r0, n, slot, hh, d0):
        src = (k_hbm, v_hbm)[kv].at[b, head, pl.ds(r0, n), :]
        dst = ring.at[slot, kv, b, hh, pl.ds(d0, n), :]
        pltpu.make_async_copy(src, dst, rsem.at[slot, kv]).start(priority=b)

    def ring_start(t, slot):
        g, c = t // CPH, t % CPH
        off = SK - W + c * R

        def inner_chunk():
            for hh in range(G):
                for kv in range(2):
                    for d0 in range(0, R, P):
                        for b in range(B):
                            kv_start(kv, b, _head_of(g, hh), off + SHIFT[kv] + d0, P, slot, hh, d0)

        def last_chunk(has_next_group):
            for hh in range(G):
                for kv in range(2):
                    keep = R - SHIFT[kv]
                    for d0 in range(0, R, P):
                        n = min(max(keep - d0, 0), P)
                        for b in range(B):
                            if n:
                                kv_start(kv, b, _head_of(g, hh), SK - keep + d0, n, slot, hh, d0)
                            if n < P and has_next_group:
                                kv_start(kv, b, _head_of(g + 1, hh), SK - W + d0 + n - keep, P - n,
                                         slot, hh, d0 + n)

        if isinstance(t, int):
            assert c < CPH - 1
            inner_chunk()
        else:
            off = pl.multiple_of(off, R)
            pl.when(c < CPH - 1)(inner_chunk)

            @pl.when(c == CPH - 1)
            def _():
                pl.when(g < NG - 1)(lambda: last_chunk(True))
                pl.when(g == NG - 1)(lambda: last_chunk(False))

    def ring_wait(t, slot):
        for kv in range(2):
            pl.when(t < NSTEP - 1)(lambda: _wait_filled(ring.at[slot, kv], rsem.at[slot, kv]))
            pl.when(t == NSTEP - 1)(lambda: _wait_filled(
                ring.at[slot, kv, :, :, pl.ds(0, R - SHIFT[kv]), :], rsem.at[slot, kv]))

    def ring_tile(slot, prev, kv, b, hh):
        if not SHIFT[kv]:
            return ring[slot, kv, b, hh]
        return jnp.concatenate([ring[prev, kv, b, hh, pl.ds(R - SHIFT[kv], SHIFT[kv]), :],
                                ring[slot, kv, b, hh, pl.ds(0, R - SHIFT[kv]), :]], axis=0)

    c_copy = pltpu.make_async_copy(c_hbm, c_v, wsem.at[0])
    x_copy = pltpu.make_async_copy(x_hbm, x_v, wsem.at[1])
    _start_all(_with_queues(_streams(_pieces(wm_hbm, wm_v, wsem.at[2], 8, 1536), 4), 1, 2))
    c_copy.start()
    x_copy.start(priority=1)
    _start_all(_with_queues(_streams(_pieces(wq_hbm, wq_v, wsem.at[3], 8, 2048), 4), 1, 2))

    w2_offsets = [sum(W2_CHUNKS[:j]) for j in range(len(W2_CHUNKS))]
    ffn = _with_queues(_interleave([_streams(_pieces(w1t_hbm, w1_v, wsem.at[0], 32, D), 2),
                                    _streams(_pieces(w3t_hbm, w3_v, wsem.at[1], 32, D), 2)]), 1, 2)
    for j, (f0, fc) in enumerate(zip(w2_offsets, W2_CHUNKS)):
        ffn += _with_queues(_pieces(w2_hbm, w2_v, wsem.at[2 + j], 32, D, f0, fc), 0, 1)
    per_step = -(-len(ffn) // DEPTH)
    ffn_batches = [ffn[j * per_step:(j + 1) * per_step] for j in range(DEPTH)]

    row = lax.broadcasted_iota(jnp.int32, (8, DH), 0)
    row_r = lax.broadcasted_iota(jnp.int32, (8, R), 0)
    row_d = lax.broadcasted_iota(jnp.int32, (8, D), 0)

    def rows8(ref):
        v = ref[...].astype(F32)
        return jnp.where(row_d % 2 == 0, v[0:1], v[1:2])

    c_copy.wait()
    c8 = rows8(c_v)
    silu_c = (c8 * jax.nn.sigmoid(c8)).astype(BF)
    x_copy.wait()
    x8 = rows8(x_v)
    _wait_filled(wm_v, wsem.at[2])
    mod = jnp.dot(silu_c, wm_v[...], preferred_element_type=F32)
    sa, ca, ga, sb, cb, gb = [mod[:, i * D:(i + 1) * D] for i in range(6)]
    h = (_layernorm(x8) * (1 + ca) + sa).astype(BF)

    for hh in range(G):
        for kv in range(2):
            for b in range(B):
                if SHIFT[kv]:
                    kv_start(kv, b, _head_of(0, hh), SK - W, SHIFT[kv], NS - 1, hh, R - SHIFT[kv])
    for t in range(DEPTH):
        ring_start(t, t)
    _wait_filled(wq_v, wsem.at[3])
    q = jnp.dot(h, wq_v[...], preferred_element_type=F32)
    for head in range(HQ):
        q_s[head] = q[:, head * DH:(head + 1) * DH]
    _start_all(_with_queues(_streams(_pieces(wo_hbm, wo_v, wsem.at[4], 32, D), 4), 1, 2))
    for kv in range(2):
        if SHIFT[kv]:
            _wait_filled(ring.at[NS - 1, kv, :, :, pl.ds(R - SHIFT[kv], SHIFT[kv]), :], rsem.at[NS - 1, kv])

    scale = DH ** -0.5

    def group(g, attn):
        qs = [q_s[_head_of(g, hh)].astype(BF) for hh in range(G)]

        def step(c, carry):
            m, l, acc = carry
            t = g * CPH + c
            slot, prev = t % NS, (t + NS - 1) % NS
            ring_wait(t, slot)
            s = None
            for hh in range(G):
                for b in range(B):
                    r = lax.dot_general(qs[hh], ring_tile(slot, prev, 0, b, hh), NT, preferred_element_type=F32)
                    s = r if s is None else jnp.where(row_r == 2 * hh + b, r, s)
            s = s * scale
            m_new = jnp.maximum(m, jnp.max(s, axis=-1, keepdims=True))
            alpha = jnp.exp(m - m_new)
            p = jnp.exp(s - m_new)
            l = alpha * l + jnp.sum(p, axis=-1, keepdims=True)
            p = p.astype(BF)
            o = None
            for hh in range(G):
                for b in range(B):
                    r = jnp.dot(p, ring_tile(slot, prev, 1, b, hh), preferred_element_type=F32)
                    o = r if o is None else jnp.where(row == 2 * hh + b, r, o)
            acc = alpha * acc + o

            pl.when(t + DEPTH < NSTEP)(lambda: ring_start(t + DEPTH, prev))

            @pl.when(t + DEPTH >= NSTEP)
            def _():
                for j in range(DEPTH):
                    pl.when(t + DEPTH == NSTEP + j)(lambda j=j: _start_all(ffn_batches[j]))

            return m_new, l, acc

        init = (jnp.full((8, 1), -jnp.inf, F32), jnp.zeros((8, 1), F32), jnp.zeros((8, DH), F32))
        _, l, acc = lax.fori_loop(0, CPH, step, init)
        o = acc / l
        pl.when(g == 0)(lambda: _wait_filled(wo_v, wsem.at[4]))
        for hh in range(G):
            lhs = jnp.where(row // 2 == hh, o, 0.0).astype(BF)
            r0 = pl.multiple_of(_head_of(g, hh) * DH, DH)
            attn = attn + jnp.dot(lhs, wo_v[pl.ds(r0, DH), :], preferred_element_type=F32)
        return attn

    a = lax.fori_loop(0, NG, group, jnp.zeros((8, D), F32))
    a = a + pltpu.roll(a, 4, 0)
    a = a + pltpu.roll(a, 2, 0)

    x1 = x8 + ga * a
    h2 = (_layernorm(x1) * (1 + cb) + sb).astype(BF)
    _wait_filled(w1_v, wsem.at[0])
    _wait_filled(w3_v, wsem.at[1])
    gate = lax.dot_general(h2, w1_v[...], NT, preferred_element_type=F32)
    up = lax.dot_general(h2, w3_v[...], NT, preferred_element_type=F32)
    act = (gate * jax.nn.sigmoid(gate) * up).astype(BF)
    y = None
    for j, (f0, fc) in enumerate(zip(w2_offsets, W2_CHUNKS)):
        _wait_filled(w2_v.at[pl.ds(f0, fc), :], wsem.at[2 + j])
        r = jnp.dot(act[:, f0:f0 + fc], w2_v[pl.ds(f0, fc), :], preferred_element_type=F32)
        y = r if y is None else y + r
    out = x1 + gb * y
    o_v[...] = out[0:B].astype(BF)
    o_copy = pltpu.make_async_copy(o_v, o_hbm, wsem.at[0])
    o_copy.start()
    o_copy.wait()


@jax.jit
def pallas_adaLN_cond__sliding_block_cached__glu_gated_swiglu__decode_kernel(
    A_x: jax.Array,
    A_k_cache: jax.Array,
    A_v_cache: jax.Array,
    A_wq: jax.Array,
    A_wo: jax.Array,
    B_x: jax.Array,
    B_w1: jax.Array,
    B_w3: jax.Array,
    B_w2: jax.Array,
    c: jax.Array,
    w_mod: jax.Array,
):
    del B_x
    assert A_x.shape == (B, 1, D) and A_k_cache.shape == A_v_cache.shape == (B, HQ, SK, DH)
    hbm = pl.BlockSpec(memory_space=pltpu.HBM)
    out = pl.pallas_call(
        _kernel,
        out_shape=jax.ShapeDtypeStruct((B, D), BF),
        in_specs=[hbm] * 10,
        out_specs=hbm,
        scratch_shapes=[
            pltpu.VMEM((B, D), BF),
            pltpu.VMEM((B, D), BF),
            pltpu.VMEM((B, D), BF),
            pltpu.VMEM((NS, 2, B, G, R, DH), BF),
            pltpu.VMEM((D, HQ * DH), BF),
            pltpu.VMEM((HQ * DH, D), BF),
            pltpu.VMEM((F, D), BF),
            pltpu.VMEM((F, D), BF),
            pltpu.VMEM((F, D), BF),
            pltpu.VMEM((D, 6 * D), BF),
            pltpu.VMEM((HQ, 8, DH), F32),
            pltpu.SemaphoreType.DMA((NS, 2)),
            pltpu.SemaphoreType.DMA((max(5, 2 + len(W2_CHUNKS)),)),
        ],
        compiler_params=pltpu.CompilerParams(
            vmem_limit_bytes=64 * 1024 * 1024,
            disable_bounds_checks=True,
            disable_semaphore_checks=True,
        ),
        name="adaln_swa_swiglu_decode",
    )(A_x.reshape(B, D), c, A_k_cache, A_v_cache, A_wq, A_wo, B_w1.T, B_w3.T, B_w2, w_mod)
    return out.reshape(B, 1, D)
```
